```python
import jax
import jax.numpy as jnp

def _softmax(x, axis=-1):
    return jax.nn.softmax(x, axis=axis)

def _gelu(x):
    return jax.nn.gelu(x, approximate=True)

def _silu(x):
    return jax.nn.silu(x)

def _sigmoid(x):
    return jax.nn.sigmoid(x)

def _layernorm(x, axis=-1, eps=1e-05):
    m = jnp.mean(x, axis=axis, keepdims=True)
    v = jnp.var(x, axis=axis, keepdims=True)
    return (x - m) / jnp.sqrt(v + eps)

def _scatter_add(tgt, idx, src, axis=0):
    return tgt.at[idx].add(src)

def _segment_sum(src, seg, n):
    return jax.ops.segment_sum(src, seg, n)

class _Rng:

    def __init__(self, key):
        self._k = key

    def _next(self):
        self._k, sub = jax.random.split(self._k)
        return sub

    def normal(self, shape):
        return jax.random.normal(self._next(), shape, dtype=jnp.bfloat16)

    def randint(self, lo, hi, shape):
        return jax.random.randint(self._next(), shape, lo, hi, dtype=jnp.int32)

    def uniform(self, shape, lo=0.0, hi=1.0):
        return jax.random.uniform(self._next(), shape, jnp.bfloat16, lo, hi)

    def permutation(self, n):
        return jax.random.permutation(self._next(), n)
kernel_name = 'sequential_preLN__memory_aug_infini_attn__moe_arch_mod__prompt'

def setup_inputs():
    _rng = _Rng(jax.random.key(int.from_bytes(__import__("os").urandom(4), "little")))
    _w = lambda a: (lambda t: t.astype(jnp.bfloat16) if jnp.issubdtype(t.dtype, jnp.floating) else t)(jnp.asarray(a))

    def _A_setup():
        B, S, D, H = (1, 2048, 576, 32)
        N = 4
        L = max(1, S // N)
        sc = D ** (-0.5)
        return {'x': _w((lambda *s: _rng.normal(s) * 0.05)(B, N * L, D)), 'wq': _w((lambda *s: _rng.normal(s) * 0.05)(D, D) * sc), 'wk': _w((lambda *s: _rng.normal(s) * 0.05)(D, D) * sc), 'wv': _w((lambda *s: _rng.normal(s) * 0.05)(D, D) * sc), 'wo': _w((lambda *s: _rng.normal(s) * 0.05)(D, D) * sc), 'beta': _w((lambda *s: _rng.normal(s) * 0.05)(H))}
    _A_in = _A_setup()

    def _B_setup():
        B, S, D, F, C = (1, 2048, 576, 4608, 1)
        return {'x': _w((lambda *s: _rng.normal(s) * 0.05)(B, S, D)), 'w_r': _w((lambda *s: _rng.normal(s) * 0.05)(D)), 'w_gate': _w((lambda *s: _rng.normal(s) * 0.05)(D, F)), 'w_up': _w((lambda *s: _rng.normal(s) * 0.05)(D, F)), 'w_down': _w((lambda *s: _rng.normal(s) * 0.05)(F, D))}
    _B_in = _B_setup()
    return {'A_x': _A_in['x'], 'A_wq': _A_in['wq'], 'A_wk': _A_in['wk'], 'A_wv': _A_in['wv'], 'A_wo': _A_in['wo'], 'A_beta': _A_in['beta'], 'B_x': _B_in['x'], 'B_w_r': _B_in['w_r'], 'B_w_gate': _B_in['w_gate'], 'B_w_up': _B_in['w_up'], 'B_w_down': _B_in['w_down']}

def reference(A_x, A_wq, A_wk, A_wv, A_wo, A_beta, B_x, B_w_r, B_w_gate, B_w_up, B_w_down):

    def _A_ref(x, wq, wk, wv, wo, beta):
        B, S, D = x.shape
        H = 32
        Dh = D // H
        N = 4
        L = S // N
        q = (lambda x, *d: x.transpose(*d))((x @ wq).reshape(B, S, H, Dh), 0, 2, 1, 3).reshape(B, H, N, L, Dh)
        k = (lambda x, *d: x.transpose(*d))((x @ wk).reshape(B, S, H, Dh), 0, 2, 1, 3).reshape(B, H, N, L, Dh)
        v = (lambda x, *d: x.transpose(*d))((x @ wv).reshape(B, S, H, Dh), 0, 2, 1, 3).reshape(B, H, N, L, Dh)
        phi = lambda t: jnp.where(t > 0, t + 1.0, jnp.exp(t))
        scale = Dh ** (-0.5)
        ar = jnp.arange(L)
        mask = (lambda x, dt: x.astype(dt))(ar[:, None] < ar[None, :], x.dtype) * -1000000000.0
        g = _sigmoid(beta).reshape(1, H, 1, 1)
        M = jnp.einsum('bhd,bhe->bhde', q[:, :, 0, 0, :] * 0.0, q[:, :, 0, 0, :] * 0.0)
        z = q[:, :, 0, 0, :] * 0.0
        outs = []
        for s in range(N):
            qs, ks, vs = (q[:, :, s].copy(), k[:, :, s].copy(), v[:, :, s].copy())
            logits = jnp.einsum('bhqd,bhkd->bhqk', qs, ks) * scale + mask
            p = _softmax(logits, axis=-1)
            a_dot = jnp.einsum('bhqk,bhkd->bhqd', p, vs)
            pq = phi(qs)
            num = jnp.einsum('bhld,bhde->bhle', pq, M)
            den = jnp.einsum('bhld,bhd->bhl', pq, z)[..., None] + 1e-06
            a_mem = num / den
            o = g * a_mem + (1.0 - g) * a_dot
            outs.append(o)
            pk = phi(ks)
            M = M + jnp.einsum('bhld,bhle->bhde', pk, vs)
            z = z + jnp.einsum('bhld->bhd', pk)
        o = (lambda x, *d: x.transpose(*d))(jnp.stack(outs, 2).reshape(B, H, S, Dh), 0, 2, 1, 3).reshape(B, S, D)
        return o @ wo

    def _B_ref(x, w_r, w_gate, w_up, w_down):
        B, S, D = x.shape
        C = 1
        r = x @ w_r
        idx = jnp.argsort(-r, axis=-1)[:, :C]
        idx_e = jnp.repeat(idx.reshape(B, C, 1), D, axis=2)
        x_sel = jnp.take_along_axis(x, idx_e, axis=1)
        g = _silu(x_sel @ w_gate)
        u = x_sel @ w_up
        y = g * u @ w_down
        r_sel = _sigmoid(jnp.take_along_axis(r, idx, axis=1))
        y = y * r_sel.reshape(B, C, 1)
        b_off = (jnp.arange(B) * S).reshape(B, 1)
        flat_idx = (idx + b_off).reshape(B * C)
        zero = (x * 0.0).reshape(B * S, D)
        upd = _scatter_add(zero, flat_idx, y.reshape(B * C, D), axis=0)
        return x + upd.reshape(B, S, D)
    x = A_x
    h = x + _A_ref(_layernorm(x, axis=-1), A_wq, A_wk, A_wv, A_wo, A_beta)
    h2 = h + _B_ref(_layernorm(h, axis=-1), B_w_r, B_w_gate, B_w_up, B_w_down)
    return h2
```

```python
import jax
import jax.numpy as jnp
import jax.experimental.pallas as pl
import jax.experimental.pallas.tpu as pltpu

S, D, H, DH, NSEG, L, F = 2048, 576, 32, 18, 4, 512, 4608
T = 128
NT = 5
DP = NT * T
HPT = (7, 7, 7, 7, 4)
LOG2E = 1.4426950408889634
QSCALE = (DH ** -0.5) * LOG2E
ROW_A = tuple((126 * t) // 8 * 8 for t in range(NT))
ROW_B = tuple(-(-min(126 * (t + 1), D) // 8) * 8 for t in range(NT))

f32, bf16 = jnp.float32, jnp.bfloat16


def _iota(shape, d):
    return jax.lax.broadcasted_iota(jnp.int32, shape, d)


def _dot(a, b):
    return jnp.dot(a, b, preferred_element_type=f32)


def _dot_nt(a, b):
    return jax.lax.dot_general(a, b, (((1,), (1,)), ((), ())), preferred_element_type=f32)


def _phi(t):
    return jnp.where(t > 0, t + 1.0, jnp.exp(t))


def _slot_rows(wt):
    z = jnp.zeros((2, wt.shape[1]), wt.dtype)
    parts = []
    for t in range(NT - 1):
        parts += [wt[126 * t:126 * (t + 1)], z]
    parts += [wt[504:576], jnp.zeros((56, wt.shape[1]), wt.dtype)]
    return jnp.concatenate(parts, axis=0)


def _layernorm_rows(x):
    mu = jnp.mean(x, axis=0, keepdims=True)
    xc = x - mu
    var = jnp.mean(xc * xc, axis=0, keepdims=True)
    return xc * jax.lax.rsqrt(var + 1e-5)


def _kernel(x_hbm, wq_hbm, wk_hbm, wv_hbm, wo_hbm, beta_ref, wr_ref, wg_hbm, wu_hbm, wd_hbm,
            out_hbm,
            x_buf, w_raw, wqT, wkT, wvT, woT, wg, wu, wd, xn, qT, k_s, phiqT, phikT, vT, oT_pad,
            mem, mask_s, gcol, wrcol, lnh_s, r_s, stage,
            x_sem, w_sem, f_sem, o_sem, p_sem):
    def x_copy(s):
        return pltpu.make_async_copy(x_hbm.at[:, pl.ds(s * L, L)], x_buf.at[s], x_sem.at[s])

    w_copies = [pltpu.make_async_copy(w, w_raw.at[i], w_sem.at[i])
                for i, w in enumerate((wv_hbm, wq_hbm, wk_hbm, wo_hbm))]
    f_copies = [pltpu.make_async_copy(a, b, f_sem.at[i])
                for i, (a, b) in enumerate(((wg_hbm, wg), (wu_hbm, wu), (wd_hbm, wd)))]
    x_copy(0).start()
    for c in w_copies:
        c.start()
    for s in range(1, NSEG):
        x_copy(s).start()
    for c in f_copies:
        c.start()

    hrow = (_iota((D, T), 0) * 3641) >> 16
    onehot = jnp.where(hrow == _iota((D, T), 1), 1.0, 0.0).astype(bf16)
    brow = jnp.concatenate([beta_ref[...].astype(f32).reshape(1, H), jnp.zeros((1, T - H), f32)], axis=1)
    bmat = jnp.broadcast_to(brow, (T, T)).T.astype(bf16)
    gcol[...] = jax.nn.sigmoid(_dot(onehot, bmat))
    wrow = jnp.concatenate([wr_ref[...].astype(f32).reshape(1, D), jnp.zeros((1, DP - D), f32)], axis=1)
    wrcol[...] = jnp.broadcast_to(wrow, (T, DP)).T[0:D]
    for t in range(NT):
        n = ROW_B[t] - ROW_A[t]
        hr = ((_iota((136, T), 0) + ROW_A[t]) * 3641) >> 16
        ln = _iota((136, T), 1)
        hc = (ln * 3641) >> 16
        ok = (hr == hc + 7 * t) & (ln < HPT[t] * DH) & (_iota((136, T), 0) < n)
        mask_s[t] = jnp.where(ok, 1.0, 0.0).astype(f32)
    mem[...] = jnp.zeros(mem.shape, f32)

    w_copies[0].wait()
    wvT[...] = w_raw[0].astype(f32).T.astype(bf16)
    w_copies[1].wait()
    wqT[...] = _slot_rows(w_raw[1].astype(f32).T).astype(bf16)
    w_copies[2].wait()
    wkT[...] = _slot_rows(w_raw[2].astype(f32).T).astype(bf16)
    w_copies[3].wait()
    woT[...] = w_raw[3].astype(f32).T.astype(bf16)

    causal = _iota((T, T), 0) <= _iota((T, T), 1)

    def out_copy(s):
        return pltpu.make_async_copy(x_buf.at[s], out_hbm.at[:, pl.ds(s * L, L)], o_sem.at[s])

    def seg_body(s, carry):
        x_copy(s).wait()
        xn[...] = _layernorm_rows(x_buf[s].astype(f32)).astype(bf16)

        vT[...] = _dot(wvT[...], xn[...])
        q = _dot(wqT[...], xn[...])
        qT[...] = (q * QSCALE).astype(bf16)
        phiqT[...] = _phi(q).astype(bf16)
        k = _dot(wkT[...], xn[...])
        phikT[...] = _phi(k).astype(bf16)
        k_s[...] = k.T.astype(bf16)

        for t in range(NT):
            nh = HPT[t]
            for j in range(4):
                R = T * (j + 1)
                qt = qT[T * t:T * (t + 1), T * j:T * (j + 1)]
                kt = k_s[0:R, T * t:T * (t + 1)]
                lk = _iota((R, T), 1)
                lhs = jnp.concatenate(
                    [jnp.where((lk >= DH * hh) & (lk < DH * (hh + 1)), kt, jnp.zeros((), bf16))
                     for hh in range(nh)], axis=0)
                st = _dot(lhs, qt)
                for hh in range(nh):
                    h = 7 * t + hh
                    sh = st[hh * R:(hh + 1) * R]
                    dg = jnp.where(causal, sh[R - T:], -jnp.inf)
                    sh = dg if j == 0 else jnp.concatenate([sh[:R - T], dg], axis=0)
                    p = jnp.exp2(sh - jnp.max(sh, axis=0, keepdims=True))
                    r0 = (DH * h) % 8
                    a = DH * h - r0
                    ones_row = DH if r0 == 0 else r0 - 1
                    vl = jnp.where(_iota((24, R), 0) == ones_row, 1.0, vT[a:a + 24, 0:R])
                    o = _dot(vl, p)
                    inv = 1.0 / o[ones_row:ones_row + 1]
                    oT_pad[24 * h:24 * h + 24, T * j:T * (j + 1)] = o * inv

        row8 = _iota((8, L), 0)
        od_rows = []
        for v in range(D // 8):
            lo, hi = 8 * v, 8 * v + 7
            hs = sorted({lo // DH, hi // DH})
            h0 = hs[0]
            off0 = 24 * h0 + (lo - (DH * h0 - (DH * h0) % 8))
            val = oT_pad[off0:off0 + 8, :]
            if len(hs) == 2:
                h1 = hs[1]
                off1 = 24 * h1 + (lo - (DH * h1 - (DH * h1) % 8))
                val = jnp.where(row8 < DH * h1 - lo, val, oT_pad[off1:off1 + 8, :])
            od_rows.append(val)
        od = jnp.concatenate(od_rows, axis=0)
        g = jnp.concatenate([gcol[...]] * 4, axis=1)
        oT_pad[0:D, :] = (1.0 - g) * od

        @pl.when(s > 0)
        def _():
            for t in range(NT):
                n = ROW_B[t] - ROW_A[t]
                nd = _dot(mem[t].astype(bf16), phiqT[T * t:T * (t + 1), :])
                am = nd[0:n] / (nd[136:136 + n] + 1e-6)
                ra = ROW_A[t]
                oT_pad[ra:ra + n, :] += jnp.concatenate([gcol[ra:ra + n, :]] * 4, axis=1) * am

        @pl.when(s < NSEG - 1)
        def _():
            ones = jnp.ones((16, L), bf16)
            for t in range(NT):
                n = ROW_B[t] - ROW_A[t]
                ra = ROW_A[t]
                pk = phikT[T * t:T * (t + 1), :]
                m = _dot_nt(vT[ra:ra + n, :].astype(bf16), pk)
                z = _dot_nt(ones, pk)[0:1]
                mk = mask_s[t, 0:n, :] > 0
                mem[t, 0:n, :] += jnp.where(mk, m, 0.0)
                mem[t, 136:136 + n, :] += jnp.where(mk, z, 0.0)

        att = _dot(woT[...], oT_pad[0:D, :].astype(bf16))
        h = x_buf[s].astype(f32) + att
        lnh = _layernorm_rows(h)
        lnh_b = lnh.astype(bf16)
        lnh_s[s] = lnh_b
        wr4 = jnp.concatenate([wrcol[...]] * 4, axis=1)
        r_s[pl.ds(s, 1), :] = jnp.sum(lnh_b.astype(f32) * wr4, axis=0, keepdims=True)
        x_buf[s] = (h + lnh).astype(bf16)
        out_copy(s).start()
        return carry

    jax.lax.fori_loop(0, NSEG, seg_body, 0)

    r = r_s[...]
    rmax = jnp.max(r)
    tok = _iota((NSEG, L), 0) * L + _iota((NSEG, L), 1)
    idx = jnp.minimum(jnp.min(jnp.where(r == rmax, tok, S)), S - 1)
    sseg = idx // L
    col = idx % L
    blk = pl.multiple_of((col // T) * T, T)
    sel = _iota((D, T), 1) == (col - blk)
    lblk = lnh_s[sseg, :, pl.ds(blk, T)].astype(f32)
    xcol = jnp.sum(jnp.where(sel, lblk, 0.0), axis=1, keepdims=True)
    xmat = jnp.concatenate([jnp.broadcast_to(xcol, (D, T)), jnp.zeros((DP - D, T), f32)], axis=0)
    xs = xmat.T[0:16, 0:D].astype(bf16)
    for c in f_copies:
        c.wait()
    gq = _dot(xs, wg[...])
    uq = _dot(xs, wu[...])
    act = (gq * jax.nn.sigmoid(gq) * uq).astype(bf16)
    y = _dot_nt(act, wd[...])
    y = y * jax.nn.sigmoid(jnp.full((1, 1), rmax, f32))
    ymat = jnp.concatenate([jnp.broadcast_to(y[0:1], (T, D)), jnp.zeros((T, DP - D), f32)], axis=1)
    ycol = ymat.T[0:D]
    for s in range(NSEG):
        out_copy(s).wait()
    oblk = x_buf[sseg, :, pl.ds(blk, T)].astype(f32)
    stage[...] = jnp.where(sel, oblk + ycol, oblk).astype(bf16)
    pc = pltpu.make_async_copy(
        stage, out_hbm.at[:, pl.ds(pl.multiple_of(sseg * L + blk, T), T)], p_sem)
    pc.start()
    pc.wait()


@jax.jit
def pallas_sequential_preLN__memory_aug_infini_attn__moe_arch_mod__prompt_kernel(
    A_x: jax.Array,
    A_wq: jax.Array,
    A_wk: jax.Array,
    A_wv: jax.Array,
    A_wo: jax.Array,
    A_beta: jax.Array,
    B_x: jax.Array,
    B_w_r: jax.Array,
    B_w_gate: jax.Array,
    B_w_up: jax.Array,
    B_w_down: jax.Array,
):
    hbm = pl.BlockSpec(memory_space=pltpu.MemorySpace.HBM)
    vm = pl.BlockSpec(memory_space=pltpu.VMEM)
    scratch = [
        pltpu.VMEM((NSEG, D, L), bf16),
        pltpu.VMEM((4, D, D), bf16),
        pltpu.VMEM((DP, D), bf16),
        pltpu.VMEM((DP, D), bf16),
        pltpu.VMEM((D, D), bf16),
        pltpu.VMEM((D, D), bf16),
        pltpu.VMEM((D, F), bf16),
        pltpu.VMEM((D, F), bf16),
        pltpu.VMEM((D, F), bf16),
        pltpu.VMEM((D, L), bf16),
        pltpu.VMEM((DP, L), bf16),
        pltpu.VMEM((L, DP), bf16),
        pltpu.VMEM((DP, L), bf16),
        pltpu.VMEM((DP, L), bf16),
        pltpu.VMEM((D, L), f32),
        pltpu.VMEM((H * 24, L), f32),
        pltpu.VMEM((NT, 272, T), f32),
        pltpu.VMEM((NT, 136, T), f32),
        pltpu.VMEM((D, T), f32),
        pltpu.VMEM((D, T), f32),
        pltpu.VMEM((NSEG, D, L), bf16),
        pltpu.VMEM((NSEG, L), f32),
        pltpu.VMEM((D, T), bf16),
        pltpu.SemaphoreType.DMA((NSEG,)),
        pltpu.SemaphoreType.DMA((4,)),
        pltpu.SemaphoreType.DMA((3,)),
        pltpu.SemaphoreType.DMA((NSEG,)),
        pltpu.SemaphoreType.DMA(()),
    ]
    out_t = pl.pallas_call(
        _kernel,
        out_shape=jax.ShapeDtypeStruct((D, S), bf16),
        in_specs=[hbm, hbm, hbm, hbm, hbm, vm, vm, hbm, hbm, hbm],
        out_specs=hbm,
        scratch_shapes=scratch,
        compiler_params=pltpu.CompilerParams(vmem_limit_bytes=100 * 1024 * 1024),
        name="infini_attn_mod_ffn",
    )(A_x.reshape(S, D).T, A_wq, A_wk, A_wv, A_wo, A_beta, B_w_r, B_w_gate, B_w_up, B_w_down.T)
    return out_t.T.reshape(1, S, D)
```

```python
import jax
import jax.numpy as jnp
import jax.experimental.pallas as pl
import jax.experimental.pallas.tpu as pltpu

S, D, H, DH, NSEG, L, F = 2048, 576, 32, 18, 4, 512, 4608
T = 128
NT = 5
DP = NT * T
HPT = (7, 7, 7, 7, 4)
LOG2E = 1.4426950408889634
QSCALE = (DH ** -0.5) * LOG2E
ROW_A = tuple((126 * t) // 8 * 8 for t in range(NT))
ROW_B = tuple(-(-min(126 * (t + 1), D) // 8) * 8 for t in range(NT))
OFF = (0, 128, 384, 768)
SROWS = 1280 + 32

f32, bf16 = jnp.float32, jnp.bfloat16


def _iota(shape, d):
    return jax.lax.broadcasted_iota(jnp.int32, shape, d)


def _dot(a, b):
    return jnp.dot(a, b, preferred_element_type=f32)


def _dot_nt(a, b):
    return jax.lax.dot_general(a, b, (((1,), (1,)), ((), ())), preferred_element_type=f32)


def _phi(t):
    return jnp.where(t > 0, t + 1.0, jnp.exp(t))


def _slot_rows(wt):
    z = jnp.zeros((2, wt.shape[1]), wt.dtype)
    parts = []
    for t in range(NT - 1):
        parts += [wt[126 * t:126 * (t + 1)], z]
    parts += [wt[504:576], jnp.zeros((56, wt.shape[1]), wt.dtype)]
    return jnp.concatenate(parts, axis=0)


def _layernorm_rows(x):
    mu = jnp.mean(x, axis=0, keepdims=True)
    xc = x - mu
    var = jnp.mean(xc * xc, axis=0, keepdims=True)
    return xc * jax.lax.rsqrt(var + 1e-5)


def _merge(main, extra):
    out, n, m, k = [], len(main), len(extra), 0
    for i, it in enumerate(main):
        while k < m and k * n <= i * m:
            out.append(extra[k])
            k += 1
        out.append(it)
    return out + extra[k:]


def _kernel(x_hbm, wq_hbm, wk_hbm, wv_hbm, wo_hbm, beta_ref, wr_ref, wg_hbm, wu_hbm, wd_hbm,
            out_hbm,
            x_buf, w_raw, wqT, wkT, wvT, woT, wg, wu, wd, xn, qT, k_s, phiqT, phikT, vT, od, am,
            sbuf, mem, mask_s, gcol, wrcol, lnh_s, r_s, stage,
            x_sem, w_sem, f_sem, o_sem, p_sem):
    def x_copy(s):
        return pltpu.make_async_copy(x_hbm.at[:, pl.ds(s * L, L)], x_buf.at[s], x_sem.at[s])

    def out_copy(s):
        return pltpu.make_async_copy(x_buf.at[s], out_hbm.at[:, pl.ds(s * L, L)], o_sem.at[s])

    w_copies = [pltpu.make_async_copy(w, w_raw.at[i], w_sem.at[i])
                for i, w in enumerate((wk_hbm, wq_hbm, wv_hbm, wo_hbm))]
    f_copies = [pltpu.make_async_copy(a, b, f_sem.at[i])
                for i, (a, b) in enumerate(((wg_hbm, wg), (wu_hbm, wu), (wd_hbm, wd)))]
    x_copy(0).start()
    for c in w_copies:
        c.start()

    hrow = (_iota((D, T), 0) * 3641) >> 16
    onehot = jnp.where(hrow == _iota((D, T), 1), 1.0, 0.0).astype(bf16)
    brow = jnp.concatenate([beta_ref[...].astype(f32).reshape(1, H), jnp.zeros((1, T - H), f32)], axis=1)
    bmat = jnp.broadcast_to(brow, (T, T)).T.astype(bf16)
    gcol[...] = jax.nn.sigmoid(_dot(onehot, bmat))
    wrow = jnp.concatenate([wr_ref[...].astype(f32).reshape(1, D), jnp.zeros((1, DP - D), f32)], axis=1)
    wrcol[...] = jnp.broadcast_to(wrow, (T, DP)).T[0:D]
    for t in range(NT):
        n = ROW_B[t] - ROW_A[t]
        hr = ((_iota((136, T), 0) + ROW_A[t]) * 3641) >> 16
        ln = _iota((136, T), 1)
        hc = (ln * 3641) >> 16
        ok = (hr == hc + 7 * t) & (ln < HPT[t] * DH) & (_iota((136, T), 0) < n)
        mask_s[t] = jnp.where(ok, 1.0, 0.0).astype(f32)

    causal = _iota((T, T), 0) <= _iota((T, T), 1)

    def ln_item(s, j):
        def f():
            if j == 0:
                x_copy(s).wait()
            x = x_buf[s, :, T * j:T * (j + 1)].astype(f32)
            xn[s % 2, :, T * j:T * (j + 1)] = _layernorm_rows(x).astype(bf16)
        return f

    def k_item(s, t):
        def f():
            k = _dot(wkT[T * t:T * (t + 1), :], xn[s % 2])
            if s < NSEG - 1:
                phikT[s % 2, T * t:T * (t + 1), :] = _phi(k).astype(bf16)
            k_s[s % 2, :, T * t:T * (t + 1)] = k.T.astype(bf16)
        return f

    def q_item(s, t):
        def f():
            q = _dot(wqT[T * t:T * (t + 1), :], xn[s % 2])
            qT[s % 2, T * t:T * (t + 1), :] = (q * QSCALE).astype(bf16)
            if s > 0:
                phiqT[s % 2, T * t:T * (t + 1), :] = _phi(q).astype(bf16)
        return f

    def v_item(s, t):
        lo = ROW_B[t - 1] if t else 0
        hi = ROW_B[t]

        def f():
            vT[s % 2, lo:hi, :] = _dot(wvT[lo:hi, :], xn[s % 2])
        return f

    def s_item(n, hh, j):
        s, t = divmod(n, NT)
        R = T * (j + 1)

        def f():
            kt = k_s[s % 2, 0:R, T * t:T * (t + 1)]
            lk = _iota((R, T), 1)
            lhs = jnp.where((lk >= DH * hh) & (lk < DH * (hh + 1)), kt, jnp.zeros((), bf16))
            sh = _dot(lhs, qT[s % 2, T * t:T * (t + 1), T * j:T * (j + 1)])
            dg = jnp.where(causal, sh[R - T:], -jnp.inf)
            sh = dg if j == 0 else jnp.concatenate([sh[:R - T], dg], axis=0)
            sbuf[n % 2, hh, OFF[j]:OFF[j] + R, :] = sh
            sbuf[n % 2, hh, 1280 + 8 * j:1288 + 8 * j, :] = jnp.broadcast_to(
                jnp.max(sh, axis=0, keepdims=True), (8, T))
        return f

    def pv_item(n, hh, j):
        s, t = divmod(n, NT)
        R = T * (j + 1)
        h = 7 * t + hh
        r0 = (DH * h) % 8
        a = DH * h - r0
        ones_row = DH if r0 == 0 else r0 - 1

        def f():
            mx = sbuf[n % 2, hh, 1280 + 8 * j:1288 + 8 * j, :]
            p = jnp.exp2(sbuf[n % 2, hh, OFF[j]:OFF[j] + R, :] - jnp.concatenate([mx] * (R // 8), axis=0))
            vl = jnp.where(_iota((24, R), 0) == ones_row, 1.0, vT[s % 2, a:a + 24, 0:R])
            o = _dot(vl, p)
            inv = (1.0 - gcol[DH * h:DH * h + 1, :]) * pl.reciprocal(
                o[ones_row:ones_row + 1], approx=True)
            o = o * inv
            row = _iota((8, T), 0)
            for v in range(3):
                lo_ok, hi_ok = max(r0 - 8 * v, 0), min(r0 + DH - 8 * v, 8)
                dst = od.at[s % 2, a + 8 * v:a + 8 * v + 8, T * j:T * (j + 1)]
                if lo_ok == 0 and hi_ok == 8:
                    dst[...] = o[8 * v:8 * v + 8]
                elif hi_ok > lo_ok:
                    pltpu.store(dst, o[8 * v:8 * v + 8], mask=(row >= lo_ok) & (row < hi_ok))
        return f

    def mread_item(s, t):
        n = ROW_B[t] - ROW_A[t]
        ra = ROW_A[t]

        def f():
            nd = _dot(mem[t].astype(bf16), phiqT[s % 2, T * t:T * (t + 1), :])
            g = jnp.concatenate([gcol[ra:ra + n, :]] * 4, axis=1)
            val = nd[0:n] * pl.reciprocal(nd[136:136 + n] + 1e-6, approx=True) * g
            if t and ra < ROW_B[t - 1]:
                am[s % 2, ra:ra + 8, :] += val[0:8]
                am[s % 2, ra + 8:ra + n, :] = val[8:]
            else:
                am[s % 2, ra:ra + n, :] = val
        return f

    def mupd_item(s, t):
        n = ROW_B[t] - ROW_A[t]
        ra = ROW_A[t]

        def f():
            pk = phikT[s % 2, T * t:T * (t + 1), :]
            m = _dot_nt(vT[s % 2, ra:ra + n, :].astype(bf16), pk)
            z = _dot_nt(jnp.ones((16, L), bf16), pk)[0:1]
            mk = mask_s[t, 0:n, :] > 0
            m = jnp.where(mk, m, 0.0)
            z = jnp.where(mk, z, 0.0)
            if s == 0:
                mem[t, 0:n, :] = m
                mem[t, 136:136 + n, :] = z
                if n < 136:
                    mem[t, n:136, :] = jnp.zeros((136 - n, T), f32)
                    mem[t, 136 + n:272, :] = jnp.zeros((136 - n, T), f32)
            else:
                mem[t, 0:n, :] += m
                mem[t, 136:136 + n, :] += z
        return f

    def out_item(s, j):
        def f():
            o = od[s % 2, :, T * j:T * (j + 1)]
            if s > 0:
                o = o + am[s % 2, :, T * j:T * (j + 1)]
            att = _dot(woT[...], o.astype(bf16))
            h = x_buf[s, :, T * j:T * (j + 1)].astype(f32) + att
            lnh = _layernorm_rows(h)
            lnh_b = lnh.astype(bf16)
            lnh_s[s, :, T * j:T * (j + 1)] = lnh_b
            r_s[s:s + 1, T * j:T * (j + 1)] = jnp.sum(
                lnh_b.astype(f32) * wrcol[...], axis=0, keepdims=True)
            x_buf[s, :, T * j:T * (j + 1)] = (h + lnh).astype(bf16)
            if j == 3:
                out_copy(s).start()
        return f

    w_copies[0].wait()
    wkT[...] = _slot_rows(w_raw[0].astype(f32).T).astype(bf16)
    for j in range(4):
        ln_item(0, j)()
    w_copies[1].wait()
    wqT[...] = _slot_rows(w_raw[1].astype(f32).T).astype(bf16)
    k_item(0, 0)()
    w_copies[2].wait()
    wvT[...] = w_raw[2].astype(f32).T.astype(bf16)
    q_item(0, 0)()
    w_copies[3].wait()
    for s in range(1, NSEG):
        x_copy(s).start()
    for c in f_copies:
        c.start()
    woT[...] = w_raw[3].astype(f32).T.astype(bf16)

    NS = NSEG * NT
    for n in range(NS + 2):
        s, t = divmod(n, NT)
        main, extra = [], []
        for j in range(4):
            nh_s = HPT[t] if n < NS else 0
            nh_p = HPT[(n - 1) % NT] if 1 <= n <= NS else 0
            for hh in range(7):
                if hh < nh_p:
                    main.append(pv_item(n - 1, hh, j))
                if hh < nh_s:
                    main.append(s_item(n, hh, j))
        s1, t1 = divmod(n + 1, NT)
        if n + 1 < NS:
            extra.append(k_item(s1, t1))
        if n < NS:
            extra.append(v_item(s, t))
        if n + 1 < NS:
            extra.append(q_item(s1, t1))
        if n < NS and s > 0:
            extra.append(mread_item(s, t))
        if 1 <= n <= NS and (n - 1) // NT < NSEG - 1:
            extra.append(mupd_item(*divmod(n - 1, NT)))
        if n < NS and s + 1 < NSEG and t in (1, 2):
            extra += [ln_item(s + 1, 2 * (t - 1)), ln_item(s + 1, 2 * (t - 1) + 1)]
        if s >= 1 and t in (1, 2) and n < NS:
            extra += [out_item(s - 1, 2 * (t - 1)), out_item(s - 1, 2 * (t - 1) + 1)]
        if n == NS + 1:
            extra += [out_item(NSEG - 1, j) for j in range(4)]
        for it in _merge(main, extra):
            it()

    r = r_s[...]
    rmax = jnp.max(r)
    tok = _iota((NSEG, L), 0) * L + _iota((NSEG, L), 1)
    idx = jnp.minimum(jnp.min(jnp.where(r == rmax, tok, S)), S - 1)
    sseg = idx // L
    col = idx % L
    blk = pl.multiple_of((col // T) * T, T)
    sel = _iota((D, T), 1) == (col - blk)
    lblk = lnh_s[sseg, :, pl.ds(blk, T)].astype(f32)
    xcol = jnp.sum(jnp.where(sel, lblk, 0.0), axis=1, keepdims=True)
    xmat = jnp.concatenate([jnp.broadcast_to(xcol, (D, T)), jnp.zeros((DP - D, T), f32)], axis=0)
    xs = xmat.T[0:16, 0:D].astype(bf16)
    for c in f_copies:
        c.wait()
    gq = _dot(xs, wg[...])
    uq = _dot(xs, wu[...])
    act = (gq * jax.nn.sigmoid(gq) * uq).astype(bf16)
    y = _dot_nt(act, wd[...])
    y = y * jax.nn.sigmoid(jnp.full((1, 1), rmax, f32))
    ymat = jnp.concatenate([jnp.broadcast_to(y[0:1], (T, D)), jnp.zeros((T, DP - D), f32)], axis=1)
    ycol = ymat.T[0:D]
    for s in range(NSEG):
        out_copy(s).wait()
    oblk = x_buf[sseg, :, pl.ds(blk, T)].astype(f32)
    stage[...] = jnp.where(sel, oblk + ycol, oblk).astype(bf16)
    pc = pltpu.make_async_copy(
        stage, out_hbm.at[:, pl.ds(pl.multiple_of(sseg * L + blk, T), T)], p_sem)
    pc.start()
    pc.wait()


@jax.jit
def pallas_sequential_preLN__memory_aug_infini_attn__moe_arch_mod__prompt_kernel(
    A_x: jax.Array,
    A_wq: jax.Array,
    A_wk: jax.Array,
    A_wv: jax.Array,
    A_wo: jax.Array,
    A_beta: jax.Array,
    B_x: jax.Array,
    B_w_r: jax.Array,
    B_w_gate: jax.Array,
    B_w_up: jax.Array,
    B_w_down: jax.Array,
):
    hbm = pl.BlockSpec(memory_space=pltpu.MemorySpace.HBM)
    vm = pl.BlockSpec(memory_space=pltpu.VMEM)
    scratch = [
        pltpu.VMEM((NSEG, D, L), bf16),
        pltpu.VMEM((4, D, D), bf16),
        pltpu.VMEM((DP, D), bf16),
        pltpu.VMEM((DP, D), bf16),
        pltpu.VMEM((D, D), bf16),
        pltpu.VMEM((D, D), bf16),
        pltpu.VMEM((D, F), bf16),
        pltpu.VMEM((D, F), bf16),
        pltpu.VMEM((D, F), bf16),
        pltpu.VMEM((2, D, L), bf16),
        pltpu.VMEM((2, DP, L), bf16),
        pltpu.VMEM((2, L, DP), bf16),
        pltpu.VMEM((2, DP, L), bf16),
        pltpu.VMEM((2, DP, L), bf16),
        pltpu.VMEM((2, D, L), f32),
        pltpu.VMEM((2, D, L), f32),
        pltpu.VMEM((2, D, L), f32),
        pltpu.VMEM((2, 7, SROWS, T), f32),
        pltpu.VMEM((NT, 272, T), f32),
        pltpu.VMEM((NT, 136, T), f32),
        pltpu.VMEM((D, T), f32),
        pltpu.VMEM((D, T), f32),
        pltpu.VMEM((NSEG, D, L), bf16),
        pltpu.VMEM((NSEG, L), f32),
        pltpu.VMEM((D, T), bf16),
        pltpu.SemaphoreType.DMA((NSEG,)),
        pltpu.SemaphoreType.DMA((4,)),
        pltpu.SemaphoreType.DMA((3,)),
        pltpu.SemaphoreType.DMA((NSEG,)),
        pltpu.SemaphoreType.DMA(()),
    ]
    out_t = pl.pallas_call(
        _kernel,
        out_shape=jax.ShapeDtypeStruct((D, S), bf16),
        in_specs=[hbm, hbm, hbm, hbm, hbm, vm, vm, hbm, hbm, hbm],
        out_specs=hbm,
        scratch_shapes=scratch,
        compiler_params=pltpu.CompilerParams(vmem_limit_bytes=110 * 1024 * 1024),
        name="infini_attn_mod_ffn",
    )(A_x.reshape(S, D).T, A_wq, A_wk, A_wv, A_wo, A_beta, B_w_r, B_w_gate, B_w_up, B_w_down.T)
    return out_t.T.reshape(1, S, D)
```

```python
import jax
import jax.numpy as jnp
import jax.experimental.pallas as pl
import jax.experimental.pallas.tpu as pltpu

S, D, H, DH, NSEG, L, F = 2048, 576, 32, 18, 4, 512, 4608
T = 128
NT = 5
DP = NT * T
HPT = (7, 7, 7, 7, 4)
LOG2E = 1.4426950408889634
QSCALE = (DH ** -0.5) * LOG2E
ROW_A = tuple((126 * t) // 8 * 8 for t in range(NT))
ROW_B = tuple(-(-min(126 * (t + 1), D) // 8) * 8 for t in range(NT))
OFF = (0, 128, 384, 768)
SROWS = 1280 + 32

f32, bf16, u32 = jnp.float32, jnp.bfloat16, jnp.uint32


def _iota(shape, d):
    return jax.lax.broadcasted_iota(jnp.int32, shape, d)


def _dot(a, b):
    return jnp.dot(a, b, preferred_element_type=f32)


def _dot_nt(a, b):
    return jax.lax.dot_general(a, b, (((1,), (1,)), ((), ())), preferred_element_type=f32)


def _pk(v):
    return pltpu.bitcast(v.astype(bf16), jnp.uint32)


def _up(v):
    return pltpu.bitcast(v, bf16)


def _phi(t):
    return jnp.where(t > 0, t + 1.0, jnp.exp(t))


def _slot_rows(wt):
    z = jnp.zeros((2, wt.shape[1]), wt.dtype)
    parts = []
    for t in range(NT - 1):
        parts += [wt[126 * t:126 * (t + 1)], z]
    parts += [wt[504:576], jnp.zeros((56, wt.shape[1]), wt.dtype)]
    return jnp.concatenate(parts, axis=0)


def _layernorm_rows(x):
    x0 = x[0:1]
    d = x - x0
    mu = jnp.mean(d, axis=0, keepdims=True)
    var = jnp.maximum(jnp.mean(d * d, axis=0, keepdims=True) - mu * mu, 0.0)
    rstd = jax.lax.rsqrt(var + 1e-5)
    return x * rstd - (x0 + mu) * rstd


def _merge(main, extra):
    out, n, m, k = [], len(main), len(extra), 0
    for i, it in enumerate(main):
        while k < m and k * n <= i * m:
            out.append(extra[k])
            k += 1
        out.append(it)
    return out + extra[k:]


def _kernel(x_hbm, wq_hbm, wk_hbm, wv_hbm, wo_hbm, beta_ref, wr_ref, wg_hbm, wu_hbm, wd_hbm,
            out_hbm,
            x_buf, w_raw, wqT, wkT, wvT, woT, wg, wu, wd, xn, qT, k_s, phiqT, phikT, vT, od, am,
            sbuf, mem, mask_s, gcol, wrcol, lnh_s, r_s, stage,
            x_sem, x0_sem, w_sem, f_sem, o_sem, p_sem):
    def x_copy(s):
        return pltpu.make_async_copy(x_hbm.at[:, pl.ds(s * L, L)], x_buf.at[s], x_sem.at[s])

    def out_copy(s):
        return pltpu.make_async_copy(x_buf.at[s], out_hbm.at[:, pl.ds(s * L, L)], o_sem.at[s])

    def x0_copy(j):
        return pltpu.make_async_copy(x_hbm.at[:, pl.ds(T * j, T)], x_buf.at[0, :, pl.ds(T * j, T)], x0_sem.at[j])

    def w_copy(i, part):
        w = (wk_hbm, wq_hbm, wv_hbm, wo_hbm)[i]
        lo, n = (0, T) if part == 0 else (T, D - T)
        return pltpu.make_async_copy(w.at[:, pl.ds(lo, n)], w_raw.at[i, :, pl.ds(lo, n)],
                                     w_sem.at[2 * i + part])

    f_copies = [pltpu.make_async_copy(a, b, f_sem.at[i])
                for i, (a, b) in enumerate(((wg_hbm, wg), (wu_hbm, wu), (wd_hbm, wd)))]
    x0_copy(0).start()
    w_copy(0, 0).start()
    x0_copy(1).start()
    w_copy(1, 0).start()
    x0_copy(2).start()
    x0_copy(3).start()
    w_copy(2, 0).start()
    for i in range(3):
        w_copy(i, 1).start()
    w_copy(3, 0).start()
    w_copy(3, 1).start()

    hrow = (_iota((D, T), 0) * 3641) >> 16
    onehot = jnp.where(hrow == _iota((D, T), 1), 1.0, 0.0).astype(bf16)
    brow = jnp.concatenate([beta_ref[...].astype(f32).reshape(1, H), jnp.zeros((1, T - H), f32)], axis=1)
    bmat = jnp.broadcast_to(brow, (T, T)).T.astype(bf16)
    gcol[...] = jax.nn.sigmoid(_dot(onehot, bmat))
    wrow = jnp.concatenate([wr_ref[...].astype(f32).reshape(1, D), jnp.zeros((1, DP - D), f32)], axis=1)
    wrcol[...] = jnp.broadcast_to(wrow, (T, DP)).T[0:D]
    for t in range(NT):
        n = ROW_B[t] - ROW_A[t]
        hr = ((_iota((136, T), 0) + ROW_A[t]) * 3641) >> 16
        ln = _iota((136, T), 1)
        hc = (ln * 3641) >> 16
        ok = (hr == hc + 7 * t) & (ln < HPT[t] * DH) & (_iota((136, T), 0) < n)
        mask_s[t] = jnp.where(ok, 1.0, 0.0).astype(f32)

    causal = _iota((T, T), 0) <= _iota((T, T), 1)

    def ln_item(s, j):
        def f():
            if s == 0:
                x0_copy(j).wait()
            elif j == 0:
                x_copy(s).wait()
            x = x_buf[s, :, T * j:T * (j + 1)].astype(f32)
            xn[s % 2, :, T * j:T * (j + 1)] = _pk(_layernorm_rows(x))
        return f

    def k_item(s, t):
        nr = T if t < NT - 1 else 80

        def f():
            k = _dot(_up(wkT[64 * t:64 * t + nr // 2, :]), _up(xn[s % 2]))
            if nr < T:
                k = jnp.concatenate([k, jnp.zeros((T - nr, L), f32)], axis=0)
            if s < NSEG - 1:
                phikT[s % 2, 64 * t:64 * (t + 1), :] = _pk(_phi(k))
            k_s[s % 2, :, T * t:T * (t + 1)] = _pk(k.T)
        return f

    def q_item(s, t):
        nr = T if t < NT - 1 else 80

        def f():
            q = _dot(_up(wqT[64 * t:64 * t + nr // 2, :]), _up(xn[s % 2]))
            if nr < T:
                q = jnp.concatenate([q, jnp.zeros((T - nr, L), f32)], axis=0)
            qT[s % 2, 64 * t:64 * (t + 1), :] = _pk(q * QSCALE)
            if s > 0:
                phiqT[s % 2, 64 * t:64 * (t + 1), :] = _pk(_phi(q))
        return f

    def v_item(s, t):
        lo = -(-ROW_B[t - 1] // 16) * 16 if t else 0
        hi = -(-ROW_B[t] // 16) * 16

        def f():
            vT[s % 2, lo:hi, :] = _dot(_up(wvT[lo // 2:hi // 2, :]), _up(xn[s % 2]))
        return f

    def s_item(n, hh, j):
        s, t = divmod(n, NT)
        R = T * (j + 1)

        def f():
            kt = k_s[s % 2, 0:R // 2, T * t:T * (t + 1)]
            lk = _iota((R // 2, T), 1)
            lhs = jnp.where((lk >= DH * hh) & (lk < DH * (hh + 1)), kt, jnp.zeros((), jnp.uint32))
            sh = _dot(_up(lhs), _up(qT[s % 2, 64 * t:64 * (t + 1), T * j:T * (j + 1)]))
            dg = jnp.where(causal, sh[R - T:], -jnp.inf)
            sh = dg if j == 0 else jnp.concatenate([sh[:R - T], dg], axis=0)
            sbuf[n % 2, hh, OFF[j]:OFF[j] + R, :] = sh
            sbuf[n % 2, hh, 1280 + 8 * j:1288 + 8 * j, :] = jnp.broadcast_to(
                jnp.max(sh, axis=0, keepdims=True), (8, T))
        return f

    def pv_item(n, hh, j):
        s, t = divmod(n, NT)
        R = T * (j + 1)
        h = 7 * t + hh
        r0 = (DH * h) % 8
        a = DH * h - r0
        ones_row = DH if r0 == 0 else r0 - 1

        def f():
            mx = sbuf[n % 2, hh, 1280 + 8 * j:1288 + 8 * j, :]
            p = jnp.exp2(sbuf[n % 2, hh, OFF[j]:OFF[j] + R, :] - jnp.concatenate([mx] * (R // 8), axis=0))
            vl = jnp.where(_iota((24, R), 0) == ones_row, 1.0, vT[s % 2, a:a + 24, 0:R])
            o = _dot(vl, p)
            inv = (1.0 - gcol[DH * h:DH * h + 1, :]) * pl.reciprocal(
                o[ones_row:ones_row + 1], approx=True)
            o = o * inv
            row = _iota((8, T), 0)
            for v in range(3):
                lo_ok, hi_ok = max(r0 - 8 * v, 0), min(r0 + DH - 8 * v, 8)
                dst = od.at[s % 2, a + 8 * v:a + 8 * v + 8, T * j:T * (j + 1)]
                if lo_ok == 0 and hi_ok == 8:
                    dst[...] = o[8 * v:8 * v + 8]
                elif hi_ok > lo_ok:
                    pltpu.store(dst, o[8 * v:8 * v + 8], mask=(row >= lo_ok) & (row < hi_ok))
        return f

    def mread_item(s, t):
        n = ROW_B[t] - ROW_A[t]
        ra = ROW_A[t]

        def f():
            lhs = mem[t].astype(bf16) if n == 136 else jnp.concatenate(
                [mem[t, 0:n], mem[t, 136:144]], axis=0).astype(bf16)
            nd = _dot(lhs, _up(phiqT[s % 2, 64 * t:64 * (t + 1), :]))
            g = jnp.concatenate([gcol[ra:ra + n, :]] * 4, axis=1)
            rd = pl.reciprocal(nd[n:n + 8] + 1e-6, approx=True)
            row = _iota((8, L), 0)
            parts = []
            for v in range(n // 8):
                lo = ra + 8 * v
                h0 = min(max(lo // DH - 7 * t, 0), HPT[t] - 1)
                h1 = min(max((lo + 7) // DH - 7 * t, 0), HPT[t] - 1)
                b = jnp.broadcast_to(rd[h0:h0 + 1], (8, L))
                if h1 != h0:
                    b = jnp.where(row < DH * (7 * t + h1) - lo, b, jnp.broadcast_to(rd[h1:h1 + 1], (8, L)))
                parts.append(b)
            val = nd[0:n] * jnp.concatenate(parts, axis=0) * g
            if t and ra < ROW_B[t - 1]:
                am[s % 2, ra:ra + 8, :] += val[0:8]
                am[s % 2, ra + 8:ra + n, :] = val[8:]
            else:
                am[s % 2, ra:ra + n, :] = val
        return f

    def mupd_item(s, t):
        n = ROW_B[t] - ROW_A[t]
        ra = ROW_A[t]

        def f():
            pk = _up(phikT[s % 2, 64 * t:64 * (t + 1), :])
            m = _dot_nt(vT[s % 2, ra:ra + n, :].astype(bf16), pk)
            z = _dot_nt(jnp.ones((16, L), bf16), pk)[0:8]
            m = jnp.where(mask_s[t, 0:n, :] > 0, m, 0.0)
            ln8 = _iota((8, T), 1)
            z = jnp.where((((ln8 * 3641) >> 16) == _iota((8, T), 0)) & (ln8 < HPT[t] * DH), z, 0.0)
            if s == 0:
                mem[t, 0:n, :] = m
                mem[t, 136:144, :] = z
            else:
                mem[t, 0:n, :] += m
                mem[t, 136:144, :] += z
        return f

    def oproj(s, j, lo, hi):
        o = od[s % 2, lo:hi, T * j:T * (j + 1)]
        if s > 0:
            o = o + am[s % 2, lo:hi, T * j:T * (j + 1)]
        return _dot(_up(woT[:, lo:hi]), o.astype(bf16))

    def out_early_item(j):
        def f():
            vT[0, :, T * j:T * (j + 1)] = oproj(NSEG - 1, j, 0, 384)
        return f

    def out_item(s, j):
        def f():
            if s == NSEG - 1:
                att = vT[0, :, T * j:T * (j + 1)] + oproj(s, j, 384, D)
            else:
                att = oproj(s, j, 0, D)
            h = x_buf[s, :, T * j:T * (j + 1)].astype(f32) + att
            lnh = _layernorm_rows(h)
            lnh_b = lnh.astype(bf16)
            lnh_s[s, :, T * j:T * (j + 1)] = lnh_b
            r_s[s:s + 1, T * j:T * (j + 1)] = jnp.sum(
                lnh_b.astype(f32) * wrcol[...], axis=0, keepdims=True)
            x_buf[s, :, T * j:T * (j + 1)] = (h + lnh).astype(bf16)
            if j == 3:
                out_copy(s).start()
        return f

    def prep_item(i, t):
        dst = (wkT, wqT, wvT, woT)[i]

        def f():
            if t < 2:
                w_copy(i, t).wait()
            if (i, t) == (3, 1):
                for s in range(1, NSEG):
                    x_copy(s).start()
                for c in f_copies:
                    c.start()
            n = min(T, D - T * t)
            wt = w_raw[i, :, T * t:T * t + n].astype(f32).T
            if i >= 2:
                dst[64 * t:64 * t + n // 2, :] = _pk(wt)
                return
            if t == 0:
                rows = wt[0:126]
            else:
                rows = jnp.concatenate([wtail[i], wt[0:126 - 2 * t]], axis=0) if t < NT - 1 else (
                    jnp.concatenate([wtail[i], wt], axis=0))
            pad = T - rows.shape[0]
            dst[64 * t:64 * (t + 1), :] = _pk(jnp.concatenate([rows, jnp.zeros((pad, D), f32)], axis=0))
            if t < NT - 1:
                m = 2 * (t + 1)
                wtail[i] = wt[T - m:T]
        return f

    wtail = {}
    prep_item(0, 0)()
    ln_item(0, 0)()
    ln_item(0, 1)()
    prep_item(1, 0)()
    ln_item(0, 2)()
    ln_item(0, 3)()
    k_item(0, 0)()
    prep_item(2, 0)()
    q_item(0, 0)()

    NS = NSEG * NT
    for n in range(NS + 2):
        s, t = divmod(n, NT)
        main, extra = [], []
        for j in range(4):
            nh_s = HPT[t] if n < NS else 0
            nh_p = HPT[(n - 1) % NT] if 1 <= n <= NS else 0
            for hh in range(7):
                if hh < nh_p:
                    main.append(pv_item(n - 1, hh, j))
                if hh < nh_s:
                    main.append(s_item(n, hh, j))
        s1, t1 = divmod(n + 1, NT)
        if n < NT - 1:
            extra += [prep_item(0, n + 1), prep_item(1, n + 1)]
        if 1 <= n < NT:
            extra.insert(0, prep_item(2, n))
        if n < NT:
            extra += [prep_item(3, n)]
        if n + 1 < NS:
            extra.append(k_item(s1, t1))
        if n < NS:
            extra.append(v_item(s, t))
        if n + 1 < NS:
            extra.append(q_item(s1, t1))
        if n < NS and s > 0:
            extra.append(mread_item(s, t))
        if 1 <= n <= NS and (n - 1) // NT < NSEG - 1:
            extra.append(mupd_item(*divmod(n - 1, NT)))
        if n < NS and s + 1 < NSEG and t in (1, 2):
            extra += [ln_item(s + 1, 2 * (t - 1)), ln_item(s + 1, 2 * (t - 1) + 1)]
        if s >= 1 and t in (1, 2) and n < NS:
            extra += [out_item(s - 1, 2 * (t - 1)), out_item(s - 1, 2 * (t - 1) + 1)]
        if n == NS:
            extra += [out_early_item(j) for j in range(4)]
        if n == NS + 1:
            extra += [out_item(NSEG - 1, j) for j in range(4)]
        for it in _merge(main, extra):
            it()

    r = r_s[...]
    rmax = jnp.max(r)
    tok = _iota((NSEG, L), 0) * L + _iota((NSEG, L), 1)
    idx = jnp.minimum(jnp.min(jnp.where(r == rmax, tok, S)), S - 1)
    sseg = idx // L
    col = idx % L
    blk = pl.multiple_of((col // T) * T, T)
    sel = _iota((D, T), 1) == (col - blk)
    lblk = lnh_s[sseg, :, pl.ds(blk, T)]
    oh16 = jnp.where(_iota((16, T), 1) == (col - blk), 1.0, 0.0).astype(bf16)
    xs = _dot_nt(oh16, lblk).astype(bf16)
    for c in f_copies:
        c.wait()
    gq = _dot(xs, wg[...])[0:8]
    uq = _dot(xs, wu[...])[0:8]
    act = (gq * jax.nn.sigmoid(gq) * uq).astype(bf16).astype(f32)
    act = jnp.concatenate([act, act], axis=0)
    ycols = []
    for v in range(D // 16):
        acc = None
        for t in range(F // T):
            term = wd[16 * v:16 * (v + 1), T * t:T * (t + 1)].astype(f32) * act[:, T * t:T * (t + 1)]
            acc = term if acc is None else acc + term
        ycols.append(jnp.sum(acc, axis=1, keepdims=True))
    ycol = jnp.concatenate(ycols, axis=0) * jax.nn.sigmoid(jnp.full((1, 1), rmax, f32))
    for s in range(NSEG):
        out_copy(s).wait()
    oblk = x_buf[sseg, :, pl.ds(blk, T)].astype(f32)
    stage[...] = jnp.where(sel, oblk + ycol, oblk).astype(bf16)
    pc = pltpu.make_async_copy(
        stage, out_hbm.at[:, pl.ds(pl.multiple_of(sseg * L + blk, T), T)], p_sem)
    pc.start()
    pc.wait()


@jax.jit
def pallas_sequential_preLN__memory_aug_infini_attn__moe_arch_mod__prompt_kernel(
    A_x: jax.Array,
    A_wq: jax.Array,
    A_wk: jax.Array,
    A_wv: jax.Array,
    A_wo: jax.Array,
    A_beta: jax.Array,
    B_x: jax.Array,
    B_w_r: jax.Array,
    B_w_gate: jax.Array,
    B_w_up: jax.Array,
    B_w_down: jax.Array,
):
    hbm = pl.BlockSpec(memory_space=pltpu.MemorySpace.HBM)
    vm = pl.BlockSpec(memory_space=pltpu.VMEM)
    scratch = [
        pltpu.VMEM((NSEG, D, L), bf16),
        pltpu.VMEM((4, D, D), bf16),
        pltpu.VMEM((DP // 2, D), u32),
        pltpu.VMEM((DP // 2, D), u32),
        pltpu.VMEM((D // 2, D), u32),
        pltpu.VMEM((D // 2, D), u32),
        pltpu.VMEM((D, F), bf16),
        pltpu.VMEM((D, F), bf16),
        pltpu.VMEM((D, F), bf16),
        pltpu.VMEM((2, D // 2, L), u32),
        pltpu.VMEM((2, DP // 2, L), u32),
        pltpu.VMEM((2, L // 2, DP), u32),
        pltpu.VMEM((2, DP // 2, L), u32),
        pltpu.VMEM((2, DP // 2, L), u32),
        pltpu.VMEM((2, D, L), f32),
        pltpu.VMEM((2, D, L), f32),
        pltpu.VMEM((2, D, L), f32),
        pltpu.VMEM((2, 7, SROWS, T), f32),
        pltpu.VMEM((NT, 144, T), f32),
        pltpu.VMEM((NT, 136, T), f32),
        pltpu.VMEM((D, T), f32),
        pltpu.VMEM((D, T), f32),
        pltpu.VMEM((NSEG, D, L), bf16),
        pltpu.VMEM((NSEG, L), f32),
        pltpu.VMEM((D, T), bf16),
        pltpu.SemaphoreType.DMA((NSEG,)),
        pltpu.SemaphoreType.DMA((4,)),
        pltpu.SemaphoreType.DMA((8,)),
        pltpu.SemaphoreType.DMA((3,)),
        pltpu.SemaphoreType.DMA((NSEG,)),
        pltpu.SemaphoreType.DMA(()),
    ]
    out_t = pl.pallas_call(
        _kernel,
        out_shape=jax.ShapeDtypeStruct((D, S), bf16),
        in_specs=[hbm, hbm, hbm, hbm, hbm, vm, vm, hbm, hbm, hbm],
        out_specs=hbm,
        scratch_shapes=scratch,
        compiler_params=pltpu.CompilerParams(vmem_limit_bytes=110 * 1024 * 1024, flags={"XLA_TPU_FORCE_LP_LLO_SCHEDULER": True}),
        name="infini_attn_mod_ffn",
    )(A_x.reshape(S, D).T, A_wq, A_wk, A_wv, A_wo, A_beta, B_w_r, B_w_gate, B_w_up, B_w_down.T)
    return out_t.T.reshape(1, S, D)
```
